```python
import jax
import jax.numpy as jnp

def _softmax(x, axis=-1):
    return jax.nn.softmax(x, axis=axis)
def _gelu(x):
    return jax.nn.gelu(x, approximate=True)
def _silu(x):
    return jax.nn.silu(x)
def _sigmoid(x):
    return jax.nn.sigmoid(x)
def _layernorm(x, axis=-1, eps=1e-5):
    m = jnp.mean(x, axis=axis, keepdims=True)
    v = jnp.var(x, axis=axis, keepdims=True)
    return (x - m) / jnp.sqrt(v + eps)
def _scatter_add(tgt, idx, src, axis=0):
    return tgt.at[idx].add(src)
def _segment_sum(src, seg, n):
    return jax.ops.segment_sum(src, seg, n)
class _Rng:
    def __init__(self, key):
        self._k = key
    def _next(self):
        self._k, sub = jax.random.split(self._k)
        return sub
    def normal(self, shape):
        return jax.random.normal(self._next(), shape, dtype=jnp.bfloat16)
    def randint(self, lo, hi, shape):
        return jax.random.randint(self._next(), shape, lo, hi, dtype=jnp.int32)
    def uniform(self, shape, lo=0.0, hi=1.0):
        return jax.random.uniform(self._next(), shape, jnp.bfloat16, lo, hi)
    def permutation(self, n):
        return jax.random.permutation(self._next(), n)


kernel_name = 'gated_mix__sliding_local_dilated__glu_gated_reglu__prompt'

def setup_inputs():
    _rng = _Rng(jax.random.key(int.from_bytes(__import__("os").urandom(4), "little")))
    _w = (lambda a: (lambda t: t.astype(jnp.bfloat16) if jnp.issubdtype(t.dtype, jnp.floating) else t)(jnp.asarray(a)))
    def _A_setup():
        B, S, D = 1, 2048, 1024
        return {
            "x": _w((lambda *s: _rng.normal(s) * 0.05)(B, S, D)),
            "wqkv": _w((lambda *s: _rng.normal(s) * 0.05)(D, 3 * D)),
            "wo": _w((lambda *s: _rng.normal(s) * 0.05)(D, D)),
        }
    _A_in = _A_setup()

    def _B_setup():
        B, S, D, F = 1, 2048, 1024, 3584
        return {
            "x": _w((lambda *s: _rng.normal(s) * 0.05)(B, S, D)),
            "W_gate": _w((lambda *s: _rng.normal(s) * 0.05)(D, F) * (2.0 / D) ** 0.5),
            "W_up": _w((lambda *s: _rng.normal(s) * 0.05)(D, F) * (2.0 / D) ** 0.5),
            "W_down": _w((lambda *s: _rng.normal(s) * 0.05)(F, D) * (1.0 / F) ** 0.5),
        }
    _B_in = _B_setup()

    return {
        "A_x": _A_in["x"],
        "A_wqkv": _A_in["wqkv"],
        "A_wo": _A_in["wo"],
        "B_x": _B_in["x"],
        "B_W_gate": _B_in["W_gate"],
        "B_W_up": _B_in["W_up"],
        "B_W_down": _B_in["W_down"],
        "gate_w": _w((lambda *s: _rng.normal(s) * 0.05)(1024)),
    }

def reference(A_x, A_wqkv, A_wo, B_x, B_W_gate, B_W_up, B_W_down, gate_w):
    def _A_ref(x, wqkv, wo):
        B, S, D = x.shape
        H = 32; Dh = D // H
        W, dil = 8, 2
        qkv = (lambda x, *d: x.transpose(*d))((x @ wqkv).reshape(B, S, 3, H, Dh), 2, 0, 3, 1, 4)
        q, k, v = qkv[0], qkv[1], qkv[2]
        scale = Dh ** -0.5
        pos = jnp.arange(S)
        off = jnp.arange(W) * dil
        idx = pos[:, None] - off[None, :]
        mask = idx >= 0
        idx_c = jnp.where(mask, idx, 0).reshape(-1)
        kg = k[:, :, idx_c, :].reshape(B, H, S, W, Dh)
        vg = v[:, :, idx_c, :].reshape(B, H, S, W, Dh)
        logits = jnp.einsum("bhsd,bhswd->bhsw", q, kg) * scale
        logits = jnp.where(mask[None, None, :, :], logits, -1e9)
        attn = _softmax(logits, axis=-1)
        o = jnp.einsum("bhsw,bhswd->bhsd", attn, vg)
        return (lambda x, *d: x.transpose(*d))(o, 0, 2, 1, 3).reshape(B, S, D) @ wo

    def _B_ref(x, W_gate, W_up, W_down):
        gate = jnp.einsum("bsd,df->bsf", x, W_gate)
        up = jnp.einsum("bsd,df->bsf", x, W_up)
        gate = gate * (lambda x, dt: x.astype(dt))(gate > 0, gate.dtype)
        h = gate * up
        return jnp.einsum("bsf,fd->bsd", h, W_down)

    x = A_x
    g = _sigmoid((x * gate_w).sum(-1, keepdims=True))
    a = _A_ref(x, A_wqkv, A_wo)
    b = _B_ref(x, B_W_gate, B_W_up, B_W_down)
    return g * a + (1 - g) * b
```

```python
import jax
import jax.numpy as jnp
import numpy as np
import jax.experimental.pallas as pl
import jax.experimental.pallas.tpu as pltpu

S, D, F = 2048, 1024, 3584
H, DH, NW, DIL = 32, 32, 8, 2
HALO = 16
f32, bf16, u32 = jnp.float32, jnp.bfloat16, jnp.uint32


def build(T=512, FC=512, RG=8):
    NB = S // T
    NC = F // FC

    def permute_rows(src32, dst32, base_src, base_dst):
        for dp in range(16):
            for cb in range(8):
                dst32[pl.ds(base_dst + dp * 32, 32), cb * 128:(cb + 1) * 128] = (
                    src32[cb, pl.ds(base_src + dp, 32, stride=16), :])

    def kern(x_hbm, wqkv_hbm, wo_hbm, wg_hbm, wu_hbm, wd_hbm, gw_hbm, o_hbm,
             x_v, o_v, wg_v, wu_v, wcat_v, wqkv_v, wt_tmp, wt_v, wo_v, gw_v, ho_v, q_v, k_v, v_v, gate_v,
             sx, sg, su, sm, so):
        def cp_x(b):
            return pltpu.make_async_copy(x_hbm.at[pl.ds(b * T, T)], x_v.at[pl.ds(b * T, T)], sx.at[b])
        def cp_g(c):
            return pltpu.make_async_copy(wg_hbm.at[:, pl.ds(c * FC, FC)], wg_v.at[:, pl.ds(c * FC, FC)], sg.at[c])
        def cp_u(c):
            return pltpu.make_async_copy(wu_hbm.at[:, pl.ds(c * FC, FC)], wu_v.at[:, pl.ds(c * FC, FC)], su.at[c])
        cp_qkv = pltpu.make_async_copy(wqkv_hbm, wqkv_v, sm.at[0])
        cp_wd = pltpu.make_async_copy(wd_hbm, wcat_v.at[pl.ds(0, F)], sm.at[1])
        cp_wo = [pltpu.make_async_copy(wo_hbm.at[:, pl.ds(j * 128, 128)], wo_v.at[j], sm.at[2]) for j in range(8)]
        cp_gw = pltpu.make_async_copy(gw_hbm, gw_v, sm.at[3])
        def cp_o(b):
            return pltpu.make_async_copy(o_v.at[pl.ds(b * T, T)], o_hbm.at[pl.ds(b * T, T)], so.at[b])

        cp_x(0).start()
        cp_gw.start()
        QPOS = 4
        for c in range(NC):
            cp_g(c).start()
            cp_u(c).start()
            if c == QPOS - 1:
                cp_qkv.start()
        cp_wd.start()
        [c_.start() for c_ in cp_wo]
        for b in range(1, NB):
            cp_x(b).start()

        lane = jax.lax.broadcasted_iota(jnp.int32, (RG, 128), 1)
        m64 = lane < 64
        m1 = (lane & 1) == 0

        def gate_calc(r0):
            xf = x_v[pl.ds(r0, T), :].astype(f32)
            gl = jnp.sum(xf * gw_v[...].astype(f32), axis=-1, keepdims=True)
            g = jax.nn.sigmoid(gl)
            gate_v[...] = jnp.broadcast_to(g, (T, 128))

        def gateup(r0, c):
            x = x_v[pl.ds(r0, T), :]
            g = jnp.dot(x, wg_v[:, c * FC:(c + 1) * FC], preferred_element_type=f32)
            u = jnp.dot(x, wu_v[:, c * FC:(c + 1) * FC], preferred_element_type=f32)
            om = 1.0 - gate_v[...]
            h = jnp.maximum(g, 0.0) * (u * jnp.tile(om, (1, FC // 128)))
            ho_v[:, c * FC:(c + 1) * FC] = h.astype(bf16)

        def transpose_w(t):
            for j in range(8):
                blk = wqkv_v[j * 128:(j + 1) * 128, t * 1024:(t + 1) * 1024]
                wt_tmp[j] = blk.T
            permute_rows(wt_tmp.bitcast(u32), wt_v.bitcast(u32), 0, t * 512)

        def qkv(r0):
            x = x_v[pl.ds(r0, T), :]
            dn = (((1,), (1,)), ((), ()))
            r = jax.lax.dot_general(x, wt_v[...], dn, preferred_element_type=f32)
            for j in range(8):
                q_v[j] = r[:, j * 128:(j + 1) * 128]
                k_v[j, HALO:, :] = r[:, 1024 + j * 128: 1024 + (j + 1) * 128]
                v_v[j, HALO:, :] = r[:, 2048 + j * 128: 2048 + (j + 1) * 128]

        def roll(a, s):
            return pltpu.roll(a, s % 128, 1)

        def attn_group(r, masked):
            lg = []
            for w in range(NW):
                acc = None
                for j in range(8):
                    p = q_v[j, pl.ds(r, RG), :] * k_v[j, pl.ds(HALO + r - DIL * w, RG), :]
                    acc = p if acc is None else acc + p
                lg.append(acc)
            st = []
            for a, b in ((0, 2), (1, 3), (4, 6), (5, 7)):
                st.append(jnp.where(m64, lg[a], lg[b]) + roll(jnp.where(m64, lg[b], lg[a]), 64))
            L = []
            for u_, v_ in ((st[0], st[1]), (st[2], st[3])):
                L.append(jnp.where(m1, u_ + roll(u_, -1), v_ + roll(v_, 1)) * (DH ** -0.5))
            if masked:
                row = jax.lax.broadcasted_iota(jnp.int32, (RG, 128), 0) + r
                wv = jnp.where(m64, 0, 2) + jnp.where(m1, 0, 1)
                L = [jnp.where(row - DIL * (wv + 4 * i) >= 0, L[i], -1e9) for i in range(2)]
            m = jnp.maximum(L[0], L[1])
            m = jnp.maximum(m, roll(m, 64))
            m = jnp.maximum(m, jnp.where(m1, roll(m, -1), roll(m, 1)))
            e = [jnp.exp(l - m) for l in L]
            s = e[0] + e[1]
            s = s + roll(s, 64)
            s = s + jnp.where(m1, roll(s, -1), roll(s, 1))
            rs = gate_v[pl.ds(r, RG), :] / s
            P = [None] * 8
            for i in range(2):
                p = e[i] * rs
                pr = roll(p, 64)
                X = [jnp.where(m64, p, pr), jnp.where(m64, pr, p)]
                for wa in range(2):
                    P[4 * i + 2 * wa] = jnp.where(m1, X[wa], roll(X[wa], 1))
                    P[4 * i + 2 * wa + 1] = jnp.where(m1, roll(X[wa], -1), X[wa])
            outs = []
            for j in range(8):
                acc = None
                for w in range(NW):
                    p = P[w] * v_v[j, pl.ds(HALO + r - DIL * w, RG), :]
                    acc = p if acc is None else acc + p
                outs.append(acc)
            return jnp.concatenate(outs, axis=1)

        def attn(first, lo, hi):
            for r in range(lo, hi, 2 * RG):
                o = jnp.concatenate([attn_group(r, first and r < HALO),
                                     attn_group(r + RG, first and r < HALO)], axis=0)
                ho_v[pl.ds(r, 2 * RG), F:] = o.astype(bf16)

        def halo_shift():
            for j in range(8):
                k_v[j, 0:HALO, :] = k_v[j, T:T + HALO, :]
                v_v[j, 0:HALO, :] = v_v[j, T:T + HALO, :]

        cp_x(0).wait()
        cp_gw.wait()
        gate_calc(0)
        for c in range(NC):
            cp_g(c).wait()
            cp_u(c).wait()
            if c == QPOS:
                cp_qkv.wait()
            gateup(0, c)
            if c >= QPOS:
                transpose_w(c - QPOS)
        qkv(0)
        for j in range(8):
            k_v[j, 0:HALO, :] = jnp.zeros((HALO, 128), f32)
            v_v[j, 0:HALO, :] = jnp.broadcast_to(v_v[j, HALO:HALO + 1, :], (HALO, 128))
        cp_wd.wait()
        [c_.wait() for c_ in cp_wo]
        permute_rows(wo_v.bitcast(u32), wcat_v.bitcast(u32), 0, F // 2)
        b = jnp.dot(ho_v[:, :F], wcat_v[:F, :], preferred_element_type=f32)
        attn(True, 0, T)
        b = b + jnp.dot(ho_v[:, F:], wcat_v[F:, :], preferred_element_type=f32)
        o_v[pl.ds(0, T), :] = b.astype(bf16)
        cp_o(0).start()

        def step(bi, _):
            r0 = pl.multiple_of(bi * T, T)
            cp_x(bi).wait()
            halo_shift()
            gate_calc(r0)
            qkv(r0)
            for c in range(NC):
                gateup(r0, c)
                lo = (c * (T // 16) // NC) * 16
                hi = ((c + 1) * (T // 16) // NC) * 16
                attn(False, lo, hi)
            out = jnp.dot(ho_v[...], wcat_v[...], preferred_element_type=f32)
            o_v[pl.ds(r0, T), :] = out.astype(bf16)
            cp_o(bi).start()

        jax.lax.fori_loop(1, NB, step, None)
        for b in range(NB):
            cp_o(b).wait()

    @jax.jit
    def f(A_x, A_wqkv, A_wo, B_x, B_W_gate, B_W_up, B_W_down, gate_w):
        anyspec = pl.BlockSpec(memory_space=pl.ANY)
        out = pl.pallas_call(
            kern,
            in_specs=[anyspec] * 7,
            out_specs=anyspec,
            out_shape=jax.ShapeDtypeStruct((S, D), bf16),
            scratch_shapes=[
                pltpu.VMEM((S, D), bf16), pltpu.VMEM((S, D), bf16),
                pltpu.VMEM((D, F), bf16), pltpu.VMEM((D, F), bf16), pltpu.VMEM((F + D, D), bf16),
                pltpu.VMEM((D, 3 * D), bf16), pltpu.VMEM((8, D, 128), bf16), pltpu.VMEM((3 * D, D), bf16),
                pltpu.VMEM((8, D, 128), bf16), pltpu.VMEM((1, D), bf16), pltpu.VMEM((T, F + D), bf16),
                pltpu.VMEM((8, T, 128), f32), pltpu.VMEM((8, T + HALO, 128), f32),
                pltpu.VMEM((8, T + HALO, 128), f32), pltpu.VMEM((T, 128), f32),
                pltpu.SemaphoreType.DMA((NB,)), pltpu.SemaphoreType.DMA((NC,)), pltpu.SemaphoreType.DMA((NC,)),
                pltpu.SemaphoreType.DMA((4,)), pltpu.SemaphoreType.DMA((NB,)),
            ],
            compiler_params=pltpu.CompilerParams(vmem_limit_bytes=110 * 2**20),
        )(A_x.reshape(S, D), A_wqkv, A_wo, B_W_gate, B_W_up, B_W_down, gate_w.reshape(1, D))
        return out.reshape(1, S, D)
    return f


pallas_gated_mix__sliding_local_dilated__glu_gated_reglu__prompt_kernel = build()
```

```python
import jax
import jax.numpy as jnp
import numpy as np
import jax.experimental.pallas as pl
import jax.experimental.pallas.tpu as pltpu

S, D, F = 2048, 1024, 3584
H, DH, NW, DIL = 32, 32, 8, 2
HALO = 16
f32, bf16, u32 = jnp.float32, jnp.bfloat16, jnp.uint32


def build(T=512, FC=512, RG=8, NOATT=0, NOTR=0, NSTEP=None):
    NB = S // T
    NC = F // FC

    def permute_rows(src32, dst32, base_src, base_dst):
        for dp in range(16):
            for cb in range(8):
                dst32[pl.ds(base_dst + dp * 32, 32), cb * 128:(cb + 1) * 128] = (
                    src32[cb, pl.ds(base_src + dp, 32, stride=16), :])

    def kern(x_hbm, wqkv_hbm, wo_hbm, wg_hbm, wu_hbm, wd_hbm, gw_hbm, o_hbm,
             x_v, o_v, wg_v, wu_v, wcat_v, wqkv_v, wt_tmp, wt_v, wo_v, gw_v, ho_v, q_v, k_v, v_v, gate_v,
             sx, sg, su, sm, so):
        def cp_x(b):
            return pltpu.make_async_copy(x_hbm.at[pl.ds(b * T, T)], x_v.at[pl.ds(b * T, T)], sx.at[b])
        def cp_g(c):
            return pltpu.make_async_copy(wg_hbm.at[:, pl.ds(c * FC, FC)], wg_v.at[:, pl.ds(c * FC, FC)], sg.at[c])
        def cp_u(c):
            return pltpu.make_async_copy(wu_hbm.at[:, pl.ds(c * FC, FC)], wu_v.at[:, pl.ds(c * FC, FC)], su.at[c])
        cp_qkv = pltpu.make_async_copy(wqkv_hbm, wqkv_v, sm.at[0])
        cp_wd = pltpu.make_async_copy(wd_hbm, wcat_v.at[pl.ds(0, F)], sm.at[1])
        cp_wo = [pltpu.make_async_copy(wo_hbm.at[:, pl.ds(j * 128, 128)], wo_v.at[j], sm.at[2]) for j in range(8)]
        cp_gw = pltpu.make_async_copy(gw_hbm, gw_v, sm.at[3])
        def cp_o(b):
            return pltpu.make_async_copy(o_v.at[pl.ds(b * T, T)], o_hbm.at[pl.ds(b * T, T)], so.at[b])

        WDP = [0, 1024, 2304, F]
        cp_wd = [pltpu.make_async_copy(wd_hbm.at[pl.ds(WDP[i], WDP[i + 1] - WDP[i])],
                                       wcat_v.at[pl.ds(WDP[i], WDP[i + 1] - WDP[i])], sm.at[1]) for i in range(3)]
        cp_qkv = [pltpu.make_async_copy(wqkv_hbm.at[:, pl.ds(t * D, D)], wqkv_v.at[:, pl.ds(t * D, D)], sm.at[4 + t])
                  for t in range(3)]
        sched = {
            -1: [cp_g(0), cp_x(0), cp_gw, cp_u(0), cp_g(1), cp_u(1)],
            0: [cp_g(2), cp_u(2), cp_qkv[0]],
            1: [cp_g(3), cp_u(3), cp_qkv[1]],
            2: [cp_g(4), cp_u(4), cp_qkv[2]],
            3: [cp_g(5), cp_u(5)] + cp_wo,
            4: [cp_g(6), cp_u(6), cp_wd[0]],
            5: [cp_wd[1], cp_x(1)],
            6: [cp_wd[2]] + [cp_x(b) for b in range(2, NB)],
        }
        for c_ in sched[-1]:
            c_.start()
        QPOS = 3

        lane = jax.lax.broadcasted_iota(jnp.int32, (RG, 128), 1)
        m64 = lane < 64
        m1 = (lane & 1) == 0

        def gate_calc(r0):
            xf = x_v[pl.ds(r0, T), :].astype(f32)
            gl = jnp.sum(xf * gw_v[...].astype(f32), axis=-1, keepdims=True)
            g = jax.nn.sigmoid(gl)
            gate_v[...] = jnp.broadcast_to(g, (T, 128))

        def gateup(r0, c):
            x = x_v[pl.ds(r0, T), :]
            g = jnp.dot(x, wg_v[:, c * FC:(c + 1) * FC], preferred_element_type=f32)
            u = jnp.dot(x, wu_v[:, c * FC:(c + 1) * FC], preferred_element_type=f32)
            om = 1.0 - gate_v[...]
            h = jnp.maximum(g, 0.0) * (u * jnp.tile(om, (1, FC // 128)))
            ho_v[:, c * FC:(c + 1) * FC] = h.astype(bf16)

        def transpose_w(t):
            for j in range(8):
                blk = wqkv_v[j * 128:(j + 1) * 128, t * 1024:(t + 1) * 1024]
                wt_tmp[j] = blk.T
            permute_rows(wt_tmp.bitcast(u32), wt_v.bitcast(u32), 0, t * 512)

        def qkv(r0):
            x = x_v[pl.ds(r0, T), :]
            dn = (((1,), (1,)), ((), ()))
            r = jax.lax.dot_general(x, wt_v[...], dn, preferred_element_type=f32)
            for j in range(8):
                q_v[j] = r[:, j * 128:(j + 1) * 128]
                k_v[j, HALO:, :] = r[:, 1024 + j * 128: 1024 + (j + 1) * 128]
                v_v[j, HALO:, :] = r[:, 2048 + j * 128: 2048 + (j + 1) * 128]

        def roll(a, s):
            return pltpu.roll(a, s % 128, 1)

        def attn_group(r, masked):
            if NOATT:
                return jnp.concatenate([q_v[j, pl.ds(r, RG), :] + k_v[j, pl.ds(r + HALO, RG), :] + v_v[j, pl.ds(r + HALO, RG), :] for j in range(8)], axis=1)
            lg = []
            for w in range(NW):
                acc = None
                for j in range(8):
                    p = q_v[j, pl.ds(r, RG), :] * k_v[j, pl.ds(HALO + r - DIL * w, RG), :]
                    acc = p if acc is None else acc + p
                lg.append(acc)
            st = []
            for a, b in ((0, 2), (1, 3), (4, 6), (5, 7)):
                st.append(jnp.where(m64, lg[a], lg[b]) + roll(jnp.where(m64, lg[b], lg[a]), 64))
            L = []
            for u_, v_ in ((st[0], st[1]), (st[2], st[3])):
                L.append(jnp.where(m1, u_ + roll(u_, -1), v_ + roll(v_, 1)) * (DH ** -0.5))
            if masked:
                row = jax.lax.broadcasted_iota(jnp.int32, (RG, 128), 0) + r
                wv = jnp.where(m64, 0, 2) + jnp.where(m1, 0, 1)
                L = [jnp.where(row - DIL * (wv + 4 * i) >= 0, L[i], -1e9) for i in range(2)]
            m = jnp.maximum(L[0], L[1])
            m = jnp.maximum(m, roll(m, 64))
            m = jnp.maximum(m, jnp.where(m1, roll(m, -1), roll(m, 1)))
            e = [jnp.exp(l - m) for l in L]
            s = e[0] + e[1]
            s = s + roll(s, 64)
            s = s + jnp.where(m1, roll(s, -1), roll(s, 1))
            rs = gate_v[pl.ds(r, RG), :] / s
            P = [None] * 8
            for i in range(2):
                p = e[i] * rs
                pr = roll(p, 64)
                X = [jnp.where(m64, p, pr), jnp.where(m64, pr, p)]
                for wa in range(2):
                    P[4 * i + 2 * wa] = jnp.where(m1, X[wa], roll(X[wa], 1))
                    P[4 * i + 2 * wa + 1] = jnp.where(m1, roll(X[wa], -1), X[wa])
            outs = []
            for j in range(8):
                acc = None
                for w in range(NW):
                    p = P[w] * v_v[j, pl.ds(HALO + r - DIL * w, RG), :]
                    acc = p if acc is None else acc + p
                outs.append(acc)
            return jnp.concatenate(outs, axis=1)

        def attn(first, lo, hi):
            for r in range(lo, hi, 2 * RG):
                o = jnp.concatenate([attn_group(r, first and r < HALO),
                                     attn_group(r + RG, first and r < HALO)], axis=0)
                ho_v[pl.ds(r, 2 * RG), F:] = o.astype(bf16)

        def halo_shift():
            for j in range(8):
                k_v[j, 0:HALO, :] = k_v[j, T:T + HALO, :]
                v_v[j, 0:HALO, :] = v_v[j, T:T + HALO, :]

        cp_x(0).wait()
        cp_gw.wait()
        gate_calc(0)
        for c in range(NC):
            cp_g(c).wait()
            cp_u(c).wait()
            if QPOS <= c < QPOS + 3:
                cp_qkv[c - QPOS].wait()
            for c_ in sched[c]:
                c_.start()
            gateup(0, c)
            if QPOS <= c < QPOS + 3 and not NOTR:
                transpose_w(c - QPOS)
        qkv(0)
        for j in range(8):
            k_v[j, 0:HALO, :] = jnp.zeros((HALO, 128), f32)
            v_v[j, 0:HALO, :] = jnp.broadcast_to(v_v[j, HALO:HALO + 1, :], (HALO, 128))
        [c_.wait() for c_ in cp_wd]
        [c_.wait() for c_ in cp_wo]
        permute_rows(wo_v.bitcast(u32), wcat_v.bitcast(u32), 0, F // 2)
        b = jnp.dot(ho_v[:, :F], wcat_v[:F, :], preferred_element_type=f32)
        attn(True, 0, T)
        b = b + jnp.dot(ho_v[:, F:], wcat_v[F:, :], preferred_element_type=f32)
        o_v[pl.ds(0, T), :] = b.astype(bf16)
        cp_o(0).start()

        def step(bi, _):
            r0 = pl.multiple_of(bi * T, T)
            cp_x(bi).wait()
            halo_shift()
            gate_calc(r0)
            qkv(r0)
            for c in range(NC):
                gateup(r0, c)
                lo = (c * (T // 16) // NC) * 16
                hi = ((c + 1) * (T // 16) // NC) * 16
                attn(False, lo, hi)
            out = jnp.dot(ho_v[...], wcat_v[...], preferred_element_type=f32)
            o_v[pl.ds(r0, T), :] = out.astype(bf16)
            cp_o(bi).start()

        jax.lax.fori_loop(1, NB if NSTEP is None else NSTEP, step, None)
        for b in range(NB if NSTEP is None else NSTEP):
            cp_o(b).wait()
        for b in range(NSTEP or NB, NB):
            cp_x(b).wait()

    @jax.jit
    def f(A_x, A_wqkv, A_wo, B_x, B_W_gate, B_W_up, B_W_down, gate_w):
        anyspec = pl.BlockSpec(memory_space=pl.ANY)
        out = pl.pallas_call(
            kern,
            in_specs=[anyspec] * 7,
            out_specs=anyspec,
            out_shape=jax.ShapeDtypeStruct((S, D), bf16),
            scratch_shapes=[
                pltpu.VMEM((S, D), bf16), pltpu.VMEM((S, D), bf16),
                pltpu.VMEM((D, F), bf16), pltpu.VMEM((D, F), bf16), pltpu.VMEM((F + D, D), bf16),
                pltpu.VMEM((D, 3 * D), bf16), pltpu.VMEM((8, D, 128), bf16), pltpu.VMEM((3 * D, D), bf16),
                pltpu.VMEM((8, D, 128), bf16), pltpu.VMEM((1, D), bf16), pltpu.VMEM((T, F + D), bf16),
                pltpu.VMEM((8, T, 128), f32), pltpu.VMEM((8, T + HALO, 128), f32),
                pltpu.VMEM((8, T + HALO, 128), f32), pltpu.VMEM((T, 128), f32),
                pltpu.SemaphoreType.DMA((NB,)), pltpu.SemaphoreType.DMA((NC,)), pltpu.SemaphoreType.DMA((NC,)),
                pltpu.SemaphoreType.DMA((7,)), pltpu.SemaphoreType.DMA((NB,)),
            ],
            compiler_params=pltpu.CompilerParams(vmem_limit_bytes=110 * 2**20),
        )(A_x.reshape(S, D), A_wqkv, A_wo, B_W_gate, B_W_up, B_W_down, gate_w.reshape(1, D))
        return out.reshape(1, S, D)
    return f


pallas_gated_mix__sliding_local_dilated__glu_gated_reglu__prompt_kernel = build()
```

```python
import jax
import jax.numpy as jnp
import numpy as np
import jax.experimental.pallas as pl
import jax.experimental.pallas.tpu as pltpu

S, D, F = 2048, 1024, 3584
H, DH, NW, DIL = 32, 32, 8, 2
HALO = 16
f32, bf16, u32 = jnp.float32, jnp.bfloat16, jnp.uint32


def build(T=512, FC=512, RG=8, NOATT=0, NOTR=0, NSTEP=None):
    NB = S // T
    NC = F // FC

    def permute_rows(src32, dst32, cb, base):
        for dp in range(16):
            dst32[cb, pl.ds(base + dp * 32, 32), :] = src32[cb, pl.ds(dp, 32, stride=16), :]

    def kern(x_hbm, wqkv_hbm, wo_hbm, wg_hbm, wu_hbm, wd_hbm, gw_hbm, o_hbm,
             x_v, o_v, wg_v, wu_v, wcat_v, wqkv_v, wop_v, tmp_v, wt_v, wo_v, gw_v, ho_v, q_v, k_v, v_v, gate_v,
             sx, sg, su, sm, so):
        def cp_x(b):
            return pltpu.make_async_copy(x_hbm.at[pl.ds(b * T, T)], x_v.at[pl.ds(b * T, T)], sx.at[b])
        def cp_g(c):
            return pltpu.make_async_copy(wg_hbm.at[:, pl.ds(c * FC, FC)], wg_v.at[:, pl.ds(c * FC, FC)], sg.at[c])
        def cp_u(c):
            return pltpu.make_async_copy(wu_hbm.at[:, pl.ds(c * FC, FC)], wu_v.at[:, pl.ds(c * FC, FC)], su.at[c])
        cp_wo = [pltpu.make_async_copy(wo_hbm.at[:, pl.ds(j * 128, 128)], wo_v.at[j], sm.at[2]) for j in range(8)]
        cp_gw = pltpu.make_async_copy(gw_hbm, gw_v, sm.at[3])
        def cp_o(b):
            return pltpu.make_async_copy(o_v.at[pl.ds(b * T, T)], o_hbm.at[pl.ds(b * T, T)], so.at[b])

        WDP = [0, 1024, 2304, F]
        cp_wd = [pltpu.make_async_copy(wd_hbm.at[pl.ds(WDP[i], WDP[i + 1] - WDP[i])],
                                       wcat_v.at[pl.ds(WDP[i], WDP[i + 1] - WDP[i])], sm.at[1]) for i in range(3)]
        cp_qkv = [pltpu.make_async_copy(wqkv_hbm.at[:, pl.ds(t * D, D)], wqkv_v.at[:, pl.ds(t * D, D)], sm.at[4 + t])
                  for t in range(3)]
        sched = {
            -1: [cp_g(0), cp_x(0), cp_gw, cp_u(0)],
            -2: [cp_g(1), cp_u(1)],
            0: [cp_g(2), cp_u(2), cp_qkv[0]],
            1: [cp_g(3), cp_u(3), cp_qkv[1]],
            2: [cp_g(4), cp_u(4), cp_qkv[2]],
            3: [cp_g(5), cp_u(5)] + cp_wo,
            4: [cp_g(6), cp_u(6), cp_wd[0]],
            5: [cp_wd[1], cp_x(1)],
            6: [cp_wd[2]] + [cp_x(b) for b in range(2, NB)],
        }
        for c_ in sched[-1]:
            c_.start()
        QPOS = 3

        lane = jax.lax.broadcasted_iota(jnp.int32, (RG, 128), 1)
        m64 = lane < 64
        m1 = (lane & 1) == 0

        def gate_calc(r0):
            xf = x_v[pl.ds(r0, T), :].astype(f32)
            gl = jnp.sum(xf * gw_v[...].astype(f32), axis=-1, keepdims=True)
            g = jax.nn.sigmoid(gl)
            gate_v[...] = jnp.broadcast_to(g, (T, 128))

        def gateup(r0, c, mid=None):
            x = x_v[pl.ds(r0, T), :]
            g = jnp.dot(x, wg_v[:, c * FC:(c + 1) * FC], preferred_element_type=f32)
            if mid is not None:
                mid()
            u = jnp.dot(x, wu_v[:, c * FC:(c + 1) * FC], preferred_element_type=f32)
            om = 1.0 - gate_v[...]
            h = jnp.maximum(g, 0.0) * (u * jnp.tile(om, (1, FC // 128)))
            ho_v[:, c * FC:(c + 1) * FC] = h.astype(bf16)
            return u

        def transpose_w(t):
            for j in range(8):
                blk = wqkv_v[j * 128:(j + 1) * 128, t * 1024:(t + 1) * 1024]
                tmp_v[j] = blk.T
                permute_rows(tmp_v.bitcast(u32), wt_v.bitcast(u32), j, t * 512)

        def qkv(r0):
            x = x_v[pl.ds(r0, T), :]
            dn = (((1,), (1,)), ((), ()))
            r = jax.lax.dot_general(x, jnp.concatenate([wt_v[j] for j in range(8)], axis=1), dn, preferred_element_type=f32)
            for j in range(8):
                q_v[j] = r[:, j * 128:(j + 1) * 128]
                k_v[j, HALO:, :] = r[:, 1024 + j * 128: 1024 + (j + 1) * 128]
                v_v[j, HALO:, :] = r[:, 2048 + j * 128: 2048 + (j + 1) * 128]

        def roll(a, s):
            return pltpu.roll(a, s % 128, 1)

        def attn_group(r, masked, dep):
            if NOATT:
                return jnp.concatenate([q_v[j, pl.ds(r, RG), :] + k_v[j, pl.ds(r + HALO, RG), :] + v_v[j, pl.ds(r + HALO, RG), :] for j in range(8)], axis=1)
            lg = []
            z = jnp.maximum(jnp.minimum(dep, 0.0), 0.0)
            qs = [q_v[j, pl.ds(r, RG), :] + z for j in range(8)]
            for w in range(NW):
                acc = None
                for j in range(8):
                    p = qs[j] * k_v[j, pl.ds(HALO + r - DIL * w, RG), :]
                    acc = p if acc is None else acc + p
                lg.append(acc)
            st = []
            for a, b in ((0, 2), (1, 3), (4, 6), (5, 7)):
                st.append(jnp.where(m64, lg[a], lg[b]) + roll(jnp.where(m64, lg[b], lg[a]), 64))
            L = []
            for u_, v_ in ((st[0], st[1]), (st[2], st[3])):
                L.append(jnp.where(m1, u_ + roll(u_, -1), v_ + roll(v_, 1)) * (DH ** -0.5))
            if masked:
                row = jax.lax.broadcasted_iota(jnp.int32, (RG, 128), 0) + r
                wv = jnp.where(m64, 0, 2) + jnp.where(m1, 0, 1)
                L = [jnp.where(row - DIL * (wv + 4 * i) >= 0, L[i], -1e9) for i in range(2)]
            m = jnp.maximum(L[0], L[1])
            m = jnp.maximum(m, roll(m, 64))
            m = jnp.maximum(m, jnp.where(m1, roll(m, -1), roll(m, 1)))
            e = [jnp.exp(l - m) for l in L]
            s = e[0] + e[1]
            s = s + roll(s, 64)
            s = s + jnp.where(m1, roll(s, -1), roll(s, 1))
            rs = gate_v[pl.ds(r, RG), :] / s
            P = [None] * 8
            for i in range(2):
                p = e[i] * rs
                pr = roll(p, 64)
                X = [jnp.where(m64, p, pr), jnp.where(m64, pr, p)]
                for wa in range(2):
                    P[4 * i + 2 * wa] = jnp.where(m1, X[wa], roll(X[wa], 1))
                    P[4 * i + 2 * wa + 1] = jnp.where(m1, roll(X[wa], -1), X[wa])
            outs = []
            for j in range(8):
                acc = None
                for w in range(NW):
                    p = P[w] * v_v[j, pl.ds(HALO + r - DIL * w, RG), :]
                    acc = p if acc is None else acc + p
                outs.append(acc)
            return jnp.concatenate(outs, axis=1)

        def attn(first, lo, hi, src, ntile):
            n = (hi - lo) // (2 * RG)
            for i, r in enumerate(range(lo, hi, 2 * RG)):
                t = i * ntile // n
                o = jnp.concatenate([attn_group(r + e * RG, first and r < HALO,
                                                src[r + e * RG:r + (e + 1) * RG, t * 128:(t + 1) * 128])
                                     for e in range(2)], axis=0)
                ho_v[pl.ds(r, 2 * RG), F:] = o.astype(bf16)

        def halo_shift():
            for j in range(8):
                k_v[j, 0:HALO, :] = k_v[j, T:T + HALO, :]
                v_v[j, 0:HALO, :] = v_v[j, T:T + HALO, :]

        cp_x(0).wait()
        cp_gw.wait()
        def mid0():
            cp_u(0).wait()
            gate_calc(0)
        for c in range(NC):
            cp_g(c).wait()
            if c == 0:
                for c_ in sched[-2]:
                    c_.start()
            else:
                cp_u(c).wait()
            if QPOS <= c < QPOS + 3:
                cp_qkv[c - QPOS].wait()
            for c_ in sched[c]:
                c_.start()
            gateup(0, c, mid0 if c == 0 else None)
            if QPOS <= c < QPOS + 3 and not NOTR:
                transpose_w(c - QPOS)
        qkv(0)
        for j in range(8):
            k_v[j, 0:HALO, :] = jnp.zeros((HALO, 128), f32)
            v_v[j, 0:HALO, :] = jnp.broadcast_to(v_v[j, HALO:HALO + 1, :], (HALO, 128))
        [c_.wait() for c_ in cp_wd]
        [c_.wait() for c_ in cp_wo]
        for j in range(8):
            permute_rows(wo_v.bitcast(u32), wop_v.bitcast(u32), j, 0)
        b = jnp.dot(ho_v[:, :F], wcat_v[...], preferred_element_type=f32)
        attn(True, 0, T, b, 7)
        b = b + jnp.dot(ho_v[:, F:], jnp.concatenate([wop_v[j] for j in range(8)], axis=1), preferred_element_type=f32)
        o_v[pl.ds(0, T), :] = b.astype(bf16)
        cp_o(0).start()

        def step(bi, _):
            r0 = pl.multiple_of(bi * T, T)
            cp_x(bi).wait()
            halo_shift()
            gate_calc(r0)
            qkv(r0)
            for c in range(NC):
                u = gateup(r0, c)
                lo = (c * (T // 16) // NC) * 16
                hi = ((c + 1) * (T // 16) // NC) * 16
                attn(False, lo, hi, u, FC // 128)
            wc = jnp.concatenate([wcat_v[...], jnp.concatenate([wop_v[j] for j in range(8)], axis=1)], axis=0)
            out = jnp.dot(ho_v[...], wc, preferred_element_type=f32)
            o_v[pl.ds(r0, T), :] = out.astype(bf16)
            cp_o(bi).start()

        jax.lax.fori_loop(1, NB if NSTEP is None else NSTEP, step, None)
        for b in range(NB if NSTEP is None else NSTEP):
            cp_o(b).wait()
        for b in range(NSTEP or NB, NB):
            cp_x(b).wait()

    @jax.jit
    def f(A_x, A_wqkv, A_wo, B_x, B_W_gate, B_W_up, B_W_down, gate_w):
        anyspec = pl.BlockSpec(memory_space=pl.ANY)
        out = pl.pallas_call(
            kern,
            in_specs=[anyspec] * 7,
            out_specs=anyspec,
            out_shape=jax.ShapeDtypeStruct((S, D), bf16),
            scratch_shapes=[
                pltpu.VMEM((S, D), bf16), pltpu.VMEM((S, D), bf16),
                pltpu.VMEM((D, F), bf16), pltpu.VMEM((D, F), bf16), pltpu.VMEM((F, D), bf16),
                pltpu.VMEM((D, 3 * D), bf16), pltpu.VMEM((8, D, 128), bf16), pltpu.VMEM((8, D, 128), bf16), pltpu.VMEM((8, 3 * D, 128), bf16),
                pltpu.VMEM((8, D, 128), bf16), pltpu.VMEM((1, D), bf16), pltpu.VMEM((T, F + D), bf16),
                pltpu.VMEM((8, T, 128), f32), pltpu.VMEM((8, T + HALO, 128), f32),
                pltpu.VMEM((8, T + HALO, 128), f32), pltpu.VMEM((T, 128), f32),
                pltpu.SemaphoreType.DMA((NB,)), pltpu.SemaphoreType.DMA((NC,)), pltpu.SemaphoreType.DMA((NC,)),
                pltpu.SemaphoreType.DMA((7,)), pltpu.SemaphoreType.DMA((NB,)),
            ],
            compiler_params=pltpu.CompilerParams(vmem_limit_bytes=110 * 2**20),
        )(A_x.reshape(S, D), A_wqkv, A_wo, B_W_gate, B_W_up, B_W_down, gate_w.reshape(1, D))
        return out.reshape(1, S, D)
    return f


pallas_gated_mix__sliding_local_dilated__glu_gated_reglu__prompt_kernel = build()
```

```python
import jax
import jax.numpy as jnp
import numpy as np
import jax.experimental.pallas as pl
import jax.experimental.pallas.tpu as pltpu

S, D, F = 2048, 1024, 3584
H, DH, NW, DIL = 32, 32, 8, 2
HALO = 16
f32, bf16, u32 = jnp.float32, jnp.bfloat16, jnp.uint32


def build(T=512, FC=512, RG=8, FL={'XLA_TPU_EVENLY_DISTRIBUTE_CRITICAL_NODES': True}, NO=4):
    NB = S // T
    NC = F // FC

    def permute_rows(src32, dst32, cb, base):
        for dp in range(16):
            dst32[cb, pl.ds(base + dp * 32, 32), :] = src32[cb, pl.ds(dp, 32, stride=16), :]

    def kern(x_hbm, wqkv_hbm, wo_hbm, wg_hbm, wu_hbm, wd_hbm, gw_hbm, o_hbm,
             x_v, o_v, wg_v, wu_v, wcat_v, wqkv_v, wop_v, tmp_v, wt_v, wo_v, gw_v, ho_v, q_v, k_v, v_v, gate_v,
             sx, sg, su, sm, so):
        def cp_x(b):
            return pltpu.make_async_copy(x_hbm.at[pl.ds(b * T, T)], x_v.at[pl.ds(b * T, T)], sx.at[b])
        def cp_g(c):
            return pltpu.make_async_copy(wg_hbm.at[:, pl.ds(c * FC, FC)], wg_v.at[:, pl.ds(c * FC, FC)], sg.at[c])
        def cp_u(c):
            return pltpu.make_async_copy(wu_hbm.at[:, pl.ds(c * FC, FC)], wu_v.at[:, pl.ds(c * FC, FC)], su.at[c])
        cp_wo = [pltpu.make_async_copy(wo_hbm.at[:, pl.ds(j * 128, 128)], wo_v.at[j], sm.at[2]) for j in range(8)]
        cp_gw = pltpu.make_async_copy(gw_hbm, gw_v, sm.at[3])
        CW = D // NO
        def cp_o(b, n):
            return pltpu.make_async_copy(o_v.at[pl.ds(b * T, T), pl.ds(n * CW, CW)],
                                         o_hbm.at[pl.ds(b * T, T), pl.ds(n * CW, CW)], so.at[b])

        WDP = [0, 1024, 2304, F]
        cp_wd = [pltpu.make_async_copy(wd_hbm.at[pl.ds(WDP[i], WDP[i + 1] - WDP[i])],
                                       wcat_v.at[pl.ds(WDP[i], WDP[i + 1] - WDP[i])], sm.at[1]) for i in range(3)]
        cp_qkv = [pltpu.make_async_copy(wqkv_hbm.at[:, pl.ds(t * D, D)], wqkv_v.at[:, pl.ds(t * D, D)], sm.at[4 + t])
                  for t in range(3)]
        sched = {
            -1: [cp_g(0), cp_x(0), cp_gw, cp_u(0)],
            -2: [cp_g(1), cp_u(1)],
            0: [cp_g(2), cp_u(2), cp_qkv[0]],
            1: [cp_g(3), cp_u(3), cp_qkv[1]],
            2: [cp_g(4), cp_u(4), cp_qkv[2]],
            3: [cp_g(5), cp_u(5)] + cp_wo,
            4: [cp_g(6), cp_u(6), cp_wd[0]],
            5: [cp_wd[1], cp_x(1)],
            6: [cp_wd[2]] + [cp_x(b) for b in range(2, NB)],
        }
        for c_ in sched[-1]:
            c_.start()
        QPOS = 3

        lane = jax.lax.broadcasted_iota(jnp.int32, (RG, 128), 1)
        m64 = lane < 64
        m1 = (lane & 1) == 0

        def gate_calc(r0):
            xf = x_v[pl.ds(r0, T), :].astype(f32)
            gl = jnp.sum(xf * gw_v[...].astype(f32).reshape(1, D), axis=-1, keepdims=True)
            g = jax.nn.sigmoid(gl)
            gate_v[...] = jnp.broadcast_to(g, (T, 128))

        def gateup(r0, c, mid=None):
            x = x_v[pl.ds(r0, T), :]
            g = jnp.dot(x, wg_v[:, c * FC:(c + 1) * FC], preferred_element_type=f32)
            if mid is not None:
                mid()
            u = jnp.dot(x, wu_v[:, c * FC:(c + 1) * FC], preferred_element_type=f32)
            om = 1.0 - gate_v[...]
            h = jnp.maximum(g, 0.0) * (u * jnp.tile(om, (1, FC // 128)))
            ho_v[:, c * FC:(c + 1) * FC] = h.astype(bf16)
            return u

        def transpose_w(t):
            for j in range(8):
                blk = wqkv_v[j * 128:(j + 1) * 128, t * 1024:(t + 1) * 1024]
                tmp_v[j] = pltpu.bitcast(blk.T, u32)
                permute_rows(tmp_v, wt_v, j, t * 512)

        def qkv(r0):
            x = x_v[pl.ds(r0, T), :]
            dn = (((1,), (1,)), ((), ()))
            r = jax.lax.dot_general(x, jnp.concatenate([pltpu.bitcast(wt_v[j], bf16) for j in range(8)], axis=1), dn, preferred_element_type=f32)
            for j in range(8):
                q_v[j] = r[:, j * 128:(j + 1) * 128]
                k_v[j, HALO:, :] = r[:, 1024 + j * 128: 1024 + (j + 1) * 128]
                v_v[j, HALO:, :] = r[:, 2048 + j * 128: 2048 + (j + 1) * 128]

        def roll(a, s):
            return pltpu.roll(a, s % 128, 1)

        def attn_group(r, masked, dep):
            lg = []
            z = jnp.maximum(jnp.minimum(dep, 0.0), 0.0)
            qs = [q_v[j, pl.ds(r, RG), :] + z for j in range(8)]
            for w in range(NW):
                acc = None
                for j in range(8):
                    p = qs[j] * k_v[j, pl.ds(HALO + r - DIL * w, RG), :]
                    acc = p if acc is None else acc + p
                lg.append(acc)
            st = []
            for a, b in ((0, 2), (1, 3), (4, 6), (5, 7)):
                st.append(jnp.where(m64, lg[a], lg[b]) + roll(jnp.where(m64, lg[b], lg[a]), 64))
            L = []
            for u_, v_ in ((st[0], st[1]), (st[2], st[3])):
                L.append(jnp.where(m1, u_ + roll(u_, -1), v_ + roll(v_, 1)) * (DH ** -0.5))
            if masked:
                row = jax.lax.broadcasted_iota(jnp.int32, (RG, 128), 0) + r
                wv = jnp.where(m64, 0, 2) + jnp.where(m1, 0, 1)
                L = [jnp.where(row - DIL * (wv + 4 * i) >= 0, L[i], -1e9) for i in range(2)]
            m = jnp.maximum(L[0], L[1])
            m = jnp.maximum(m, roll(m, 64))
            m = jnp.maximum(m, jnp.where(m1, roll(m, -1), roll(m, 1)))
            e = [jnp.exp(l - m) for l in L]
            s = e[0] + e[1]
            s = s + roll(s, 64)
            s = s + jnp.where(m1, roll(s, -1), roll(s, 1))
            rs = gate_v[pl.ds(r, RG), :] / s
            P = [None] * 8
            for i in range(2):
                p = e[i] * rs
                pr = roll(p, 64)
                X = [jnp.where(m64, p, pr), jnp.where(m64, pr, p)]
                for wa in range(2):
                    P[4 * i + 2 * wa] = jnp.where(m1, X[wa], roll(X[wa], 1))
                    P[4 * i + 2 * wa + 1] = jnp.where(m1, roll(X[wa], -1), X[wa])
            outs = []
            for j in range(8):
                acc = None
                for w in range(NW):
                    p = P[w] * v_v[j, pl.ds(HALO + r - DIL * w, RG), :]
                    acc = p if acc is None else acc + p
                outs.append(acc)
            return jnp.concatenate(outs, axis=1)

        def attn(first, lo, hi, src, ntile):
            n = (hi - lo) // (2 * RG)
            for i, r in enumerate(range(lo, hi, 2 * RG)):
                t = i * ntile // n
                o = jnp.concatenate([attn_group(r + e * RG, first and r < HALO,
                                                src[r + e * RG:r + (e + 1) * RG, t * 128:(t + 1) * 128])
                                     for e in range(2)], axis=0)
                ho_v[pl.ds(r, 2 * RG), F:] = o.astype(bf16)

        def halo_shift():
            for j in range(8):
                k_v[j, 0:HALO, :] = k_v[j, T:T + HALO, :]
                v_v[j, 0:HALO, :] = v_v[j, T:T + HALO, :]

        cp_x(0).wait()
        cp_gw.wait()
        def mid0():
            cp_u(0).wait()
            gate_calc(0)
        for c in range(NC):
            cp_g(c).wait()
            if c == 0:
                for c_ in sched[-2]:
                    c_.start()
            else:
                cp_u(c).wait()
            if QPOS <= c < QPOS + 3:
                cp_qkv[c - QPOS].wait()
            for c_ in sched[c]:
                c_.start()
            gateup(0, c, mid0 if c == 0 else None)
            if QPOS <= c < QPOS + 3:
                transpose_w(c - QPOS)
        qkv(0)
        for j in range(8):
            k_v[j, 0:HALO, :] = jnp.zeros((HALO, 128), f32)
            v_v[j, 0:HALO, :] = jnp.broadcast_to(v_v[j, HALO:HALO + 1, :], (HALO, 128))
        [c_.wait() for c_ in cp_wd]
        [c_.wait() for c_ in cp_wo]
        for j in range(8):
            tmp_v[j] = pltpu.bitcast(wo_v[j], u32)
            permute_rows(tmp_v, wop_v, j, 0)
        b = jnp.dot(ho_v[:, :F], wcat_v[...], preferred_element_type=f32)
        attn(True, 0, T, b, 7)
        b = b + jnp.dot(ho_v[:, F:], jnp.concatenate([pltpu.bitcast(wop_v[j], bf16) for j in range(8)], axis=1), preferred_element_type=f32)
        o_v[pl.ds(0, T), :] = b.astype(bf16)
        [cp_o(0, n).start() for n in range(NO)]

        def step(bi, _):
            r0 = pl.multiple_of(bi * T, T)
            cp_x(bi).wait()
            halo_shift()
            gate_calc(r0)
            qkv(r0)
            for c in range(NC):
                u = gateup(r0, c)
                lo = (c * (T // 16) // NC) * 16
                hi = ((c + 1) * (T // 16) // NC) * 16
                attn(False, lo, hi, u, FC // 128)
            wc = jnp.concatenate([wcat_v[...], jnp.concatenate([pltpu.bitcast(wop_v[j], bf16) for j in range(8)], axis=1)], axis=0)
            for n in range(NO):
                out = jnp.dot(ho_v[...], wc[:, n * CW:(n + 1) * CW], preferred_element_type=f32)
                o_v[pl.ds(r0, T), n * CW:(n + 1) * CW] = out.astype(bf16)
                cp_o(bi, n).start()

        jax.lax.fori_loop(1, NB, step, None)
        for b in range(NB):
            [cp_o(b, n).wait() for n in range(NO)]

    @jax.jit
    def f(A_x, A_wqkv, A_wo, B_x, B_W_gate, B_W_up, B_W_down, gate_w):
        anyspec = pl.BlockSpec(memory_space=pl.ANY)
        out = pl.pallas_call(
            kern,
            in_specs=[anyspec] * 7,
            out_specs=anyspec,
            out_shape=jax.ShapeDtypeStruct((S, D), bf16),
            scratch_shapes=[
                pltpu.VMEM((S, D), bf16), pltpu.VMEM((S, D), bf16),
                pltpu.VMEM((D, F), bf16), pltpu.VMEM((D, F), bf16), pltpu.VMEM((F, D), bf16),
                pltpu.VMEM((D, 3 * D), bf16), pltpu.VMEM((8, D // 2, 128), u32), pltpu.VMEM((8, D // 2, 128), u32), pltpu.VMEM((8, 3 * D // 2, 128), u32),
                pltpu.VMEM((8, D, 128), bf16), pltpu.VMEM((D,), bf16), pltpu.VMEM((T, F + D), bf16),
                pltpu.VMEM((8, T, 128), f32), pltpu.VMEM((8, T + HALO, 128), f32),
                pltpu.VMEM((8, T + HALO, 128), f32), pltpu.VMEM((T, 128), f32),
                pltpu.SemaphoreType.DMA((NB,)), pltpu.SemaphoreType.DMA((NC,)), pltpu.SemaphoreType.DMA((NC,)),
                pltpu.SemaphoreType.DMA((7,)), pltpu.SemaphoreType.DMA((NB,)),
            ],
            compiler_params=pltpu.CompilerParams(vmem_limit_bytes=110 * 2**20, flags=FL),
        )(A_x.reshape(S, D), A_wqkv, A_wo, B_W_gate, B_W_up, B_W_down, gate_w)
        return out.reshape(1, S, D)
    return f


pallas_gated_mix__sliding_local_dilated__glu_gated_reglu__prompt_kernel = build()
```
